```python
import os as _os
_os.environ.setdefault("JAX_PLATFORMS", "cpu")
import jax
import jax.numpy as jnp

def _softmax(x, axis=-1):
    return jax.nn.softmax(x, axis=axis)
def _gelu(x):
    return jax.nn.gelu(x, approximate=True)
def _silu(x):
    return jax.nn.silu(x)
def _sigmoid(x):
    return jax.nn.sigmoid(x)
def _layernorm(x, axis=-1, eps=1e-5):
    m = jnp.mean(x, axis=axis, keepdims=True)
    v = jnp.var(x, axis=axis, keepdims=True)
    return (x - m) / jnp.sqrt(v + eps)
def _scatter_add(tgt, idx, src, axis=0):
    return tgt.at[idx].add(src)
def _segment_sum(src, seg, n):
    return jax.ops.segment_sum(src, seg, n)
class _Rng:
    def __init__(self, key):
        self._k = key
    def _next(self):
        self._k, sub = jax.random.split(self._k)
        return sub
    def normal(self, shape):
        return jax.random.normal(self._next(), shape, dtype=jnp.bfloat16)
    def randint(self, lo, hi, shape):
        return jax.random.randint(self._next(), shape, lo, hi, dtype=jnp.int32)
    def uniform(self, shape, lo=0.0, hi=1.0):
        return jax.random.uniform(self._next(), shape, jnp.bfloat16, lo, hi)
    def permutation(self, n):
        return jax.random.permutation(self._next(), n)


kernel_name = 'standalone__mha_softmax__near_ridge'

def setup_inputs():
    _rng = _Rng(jax.random.key(int.from_bytes(__import__("os").urandom(4), "little")))
    _w = (lambda a: (lambda t: t.astype(jnp.bfloat16) if jnp.issubdtype(t.dtype, jnp.floating) else t)(jnp.asarray(a)))
    B, H, Sq, Sk, D = 16, 16, 256, 256, 256
    return {
        "q": _w((lambda *s: _rng.normal(s) * 0.4)(B, H, Sq, D)),
        "k": _w((lambda *s: _rng.normal(s) * 0.4)(B, H, Sk, D)),
        "v": _w((lambda *s: _rng.normal(s) * 0.05)(B, H, Sk, D)),
    }

def reference(q, k, v):
    scale = q.shape[-1] ** -0.5
    scores = jnp.einsum("bhqd,bhkd->bhqk", q, k) * scale
    p = _softmax(scores, axis=-1)
    return jnp.einsum("bhqk,bhkd->bhqd", p, v)
```

```python
import functools

import jax
import jax.numpy as jnp
from jax import lax
from jax.experimental import pallas as pl
from jax.experimental.pallas import tpu as pltpu

_NT = (((1,), (1,)), ((), ()))
_NN = (((1,), (0,)), ((), ()))


def _mha_kernel(q_ref, k_ref, v_ref, o_ref, *, heads_per_step, scale):
    for h in range(heads_per_step):
        q = q_ref[h]
        k = k_ref[h]
        v = v_ref[h]
        s = lax.dot_general(q, k, _NT, preferred_element_type=jnp.float32) * scale
        m = jnp.max(s, axis=-1, keepdims=True)
        p = jnp.exp(s - m)
        l = jnp.sum(p, axis=-1, keepdims=True)
        o = lax.dot_general(
            p.astype(v.dtype), v, _NN, preferred_element_type=jnp.float32
        )
        o_ref[h] = (o / l).astype(o_ref.dtype)


def _mha(q, k, v, *, heads_per_step=8):
    b, h, sq, d = q.shape
    sk = k.shape[2]
    n = b * h
    q3 = q.reshape(n, sq, d)
    k3 = k.reshape(n, sk, d)
    v3 = v.reshape(n, sk, d)
    hb = heads_per_step
    assert n % hb == 0
    kernel = functools.partial(
        _mha_kernel, heads_per_step=hb, scale=float(d) ** -0.5
    )
    out = pl.pallas_call(
        kernel,
        out_shape=jax.ShapeDtypeStruct((n, sq, d), q.dtype),
        grid=(n // hb,),
        in_specs=[
            pl.BlockSpec((hb, sq, d), lambda i: (i, 0, 0)),
            pl.BlockSpec((hb, sk, d), lambda i: (i, 0, 0)),
            pl.BlockSpec((hb, sk, d), lambda i: (i, 0, 0)),
        ],
        out_specs=pl.BlockSpec((hb, sq, d), lambda i: (i, 0, 0)),
        compiler_params=pltpu.CompilerParams(
            dimension_semantics=("arbitrary",),
        ),
    )(q3, k3, v3)
    return out.reshape(b, h, sq, d)


@jax.jit
def pallas_standalone__mha_softmax__near_ridge_kernel(
    q: jax.Array,
    k: jax.Array,
    v: jax.Array,
):
    return _mha(q, k, v)
```

```python
import functools

import jax
import jax.numpy as jnp
from jax import lax
from jax.experimental import pallas as pl
from jax.experimental.pallas import tpu as pltpu

_NT = (((1,), (1,)), ((), ()))
_NN = (((1,), (0,)), ((), ()))

_MAX_HEADS_PER_STEP = 8
_VMEM_LIMIT_BYTES = 64 * 1024 * 1024


def _attend_one_head(q, k, v, scale, out_dtype):
    s = lax.dot_general(q, k, _NT, preferred_element_type=jnp.float32) * scale
    m = jnp.max(s, axis=-1, keepdims=True)
    p = jnp.exp(s - m)
    l = jnp.sum(p, axis=-1, keepdims=True)
    o = lax.dot_general(p.astype(v.dtype), v, _NN, preferred_element_type=jnp.float32)
    return (o / l).astype(out_dtype)


def _mha_kernel(q_ref, k_ref, v_ref, o_hbm, acc_ref, sem, *, hb, n_heads, scale):
    step = pl.program_id(0)
    n_steps = n_heads // hb
    is_last = step == n_steps - 1
    first = step * hb

    def flush(blk):
        rows = pl.ds(blk * hb, hb)
        return pltpu.make_async_copy(acc_ref.at[rows], o_hbm.at[rows], sem.at[0])

    def for_blocks(lo, hi, fn):
        def body(blk, carry):
            fn(flush(blk))
            return carry

        lax.fori_loop(lo, hi, body, 0)

    @pl.when(is_last)
    def _():
        for_blocks(0, n_steps - 1, lambda dma: dma.start())

    for h in range(hb):
        acc_ref[first + h] = _attend_one_head(
            q_ref[h], k_ref[h], v_ref[h], scale, acc_ref.dtype
        )

    @pl.when(is_last)
    def _():
        flush(n_steps - 1).start()
        for_blocks(0, n_steps, lambda dma: dma.wait())


def _mha(q, k, v):
    b, h, sq, d = q.shape
    sk = k.shape[2]
    n_heads = b * h
    hb = max(c for c in range(1, _MAX_HEADS_PER_STEP + 1) if n_heads % c == 0)
    kernel = functools.partial(
        _mha_kernel, hb=hb, n_heads=n_heads, scale=float(d) ** -0.5
    )
    out = pl.pallas_call(
        kernel,
        out_shape=jax.ShapeDtypeStruct((n_heads, sq, d), q.dtype),
        grid=(n_heads // hb,),
        in_specs=[
            pl.BlockSpec((hb, sq, d), lambda i: (i, 0, 0)),
            pl.BlockSpec((hb, sk, d), lambda i: (i, 0, 0)),
            pl.BlockSpec((hb, sk, d), lambda i: (i, 0, 0)),
        ],
        out_specs=pl.BlockSpec(memory_space=pl.ANY),
        scratch_shapes=[
            pltpu.VMEM((n_heads, sq, d), q.dtype),
            pltpu.SemaphoreType.DMA((1,)),
        ],
        compiler_params=pltpu.CompilerParams(
            dimension_semantics=("arbitrary",),
            vmem_limit_bytes=_VMEM_LIMIT_BYTES,
        ),
    )(
        q.reshape(n_heads, sq, d),
        k.reshape(n_heads, sk, d),
        v.reshape(n_heads, sk, d),
    )
    return out.reshape(b, h, sq, d)


@jax.jit
def pallas_standalone__mha_softmax__near_ridge_kernel(
    q: jax.Array,
    k: jax.Array,
    v: jax.Array,
):
    return _mha(q, k, v)
```

```python
import functools

import jax
import jax.numpy as jnp
from jax import lax
from jax.experimental import pallas as pl
from jax.experimental.pallas import tpu as pltpu

_NT = (((1,), (1,)), ((), ()))
_NN = (((1,), (0,)), ((), ()))

_MAX_HEADS_PER_STEP = 8
_FLUSH_ROWS = 64
_VMEM_LIMIT_BYTES = 64 * 1024 * 1024


def _attend_one_head(q, k, v, scale, out_dtype):
    s = lax.dot_general(q, k, _NT, preferred_element_type=jnp.float32) * scale
    m = jnp.max(s, axis=-1, keepdims=True)
    p = jnp.exp(s - m)
    l = jnp.sum(p, axis=-1, keepdims=True)
    o = lax.dot_general(p.astype(v.dtype), v, _NN, preferred_element_type=jnp.float32)
    return (o / l).astype(out_dtype)


def _mha_kernel(q_ref, k_ref, v_ref, o_hbm, acc_ref, sem, *, scale, rows):
    n_steps, hb, sq, _ = acc_ref.shape
    step = pl.program_id(0)
    is_last = step == n_steps - 1

    def bulk_flushes():
        blocks = pl.ds(0, n_steps - 1)
        return [
            pltpu.make_async_copy(
                acc_ref.at[blocks, j, pl.ds(r0, rows)],
                o_hbm.at[blocks, j, pl.ds(r0, rows)],
                sem.at[0],
            )
            for r0 in range(0, sq, rows)
            for j in range(hb)
        ]

    def last_flush():
        return pltpu.make_async_copy(
            acc_ref.at[n_steps - 1], o_hbm.at[n_steps - 1], sem.at[0]
        )

    if n_steps > 1:

        @pl.when(is_last)
        def _():
            for dma in bulk_flushes():
                dma.start()

    for h in range(hb):
        acc_ref[step, h] = _attend_one_head(
            q_ref[h], k_ref[h], v_ref[h], scale, acc_ref.dtype
        )

    @pl.when(is_last)
    def _():
        last_flush().start()
        if n_steps > 1:
            for dma in bulk_flushes():
                dma.wait()
        last_flush().wait()


def _mha(q, k, v):
    b, h, sq, d = q.shape
    sk = k.shape[2]
    n_heads = b * h
    hb = max(c for c in range(1, _MAX_HEADS_PER_STEP + 1) if n_heads % c == 0)
    n_steps = n_heads // hb
    rows = _FLUSH_ROWS if sq % _FLUSH_ROWS == 0 else sq
    kernel = functools.partial(_mha_kernel, scale=float(d) ** -0.5, rows=rows)
    out = pl.pallas_call(
        kernel,
        out_shape=jax.ShapeDtypeStruct((n_steps, hb, sq, d), q.dtype),
        grid=(n_steps,),
        in_specs=[
            pl.BlockSpec((hb, sq, d), lambda i: (i, 0, 0)),
            pl.BlockSpec((hb, sk, d), lambda i: (i, 0, 0)),
            pl.BlockSpec((hb, sk, d), lambda i: (i, 0, 0)),
        ],
        out_specs=pl.BlockSpec(memory_space=pl.ANY),
        scratch_shapes=[
            pltpu.VMEM((n_steps, hb, sq, d), q.dtype),
            pltpu.SemaphoreType.DMA((1,)),
        ],
        compiler_params=pltpu.CompilerParams(
            dimension_semantics=("arbitrary",),
            vmem_limit_bytes=_VMEM_LIMIT_BYTES,
        ),
    )(
        q.reshape(n_heads, sq, d),
        k.reshape(n_heads, sk, d),
        v.reshape(n_heads, sk, d),
    )
    return out.reshape(b, h, sq, d)


@jax.jit
def pallas_standalone__mha_softmax__near_ridge_kernel(
    q: jax.Array,
    k: jax.Array,
    v: jax.Array,
):
    return _mha(q, k, v)
```
